```python
import os as _os
_os.environ.setdefault('JAX_PLATFORMS', 'cpu')
import jax
import jax.numpy as jnp

def _softmax(x, axis=-1):
    return jax.nn.softmax(x, axis=axis)

def _gelu(x):
    return jax.nn.gelu(x, approximate=True)

def _silu(x):
    return jax.nn.silu(x)

def _sigmoid(x):
    return jax.nn.sigmoid(x)

def _layernorm(x, axis=-1, eps=1e-05):
    m = jnp.mean(x, axis=axis, keepdims=True)
    v = jnp.var(x, axis=axis, keepdims=True)
    return (x - m) / jnp.sqrt(v + eps)

def _scatter_add(tgt, idx, src, axis=0):
    return tgt.at[idx].add(src)

def _segment_sum(src, seg, n):
    return jax.ops.segment_sum(src, seg, n)

class _Rng:

    def __init__(self, key):
        self._k = key

    def _next(self):
        self._k, sub = jax.random.split(self._k)
        return sub

    def normal(self, shape):
        return jax.random.normal(self._next(), shape, dtype=jnp.bfloat16)

    def randint(self, lo, hi, shape):
        return jax.random.randint(self._next(), shape, lo, hi, dtype=jnp.int32)

    def uniform(self, shape, lo=0.0, hi=1.0):
        return jax.random.uniform(self._next(), shape, jnp.bfloat16, lo, hi)

    def permutation(self, n):
        return jax.random.permutation(self._next(), n)
kernel_name = 'adaLN_cond__sliding_local_dilated__dense_activation_relu__prompt'

def setup_inputs():
    _rng = _Rng(jax.random.key(int.from_bytes(__import__("os").urandom(4), "little")))
    _w = lambda a: (lambda t: t.astype(jnp.bfloat16) if jnp.issubdtype(t.dtype, jnp.floating) else t)(jnp.asarray(a))

    def _A_setup():
        B, S, D = (1, 2048, 576)
        return {'x': _w((lambda *s: _rng.normal(s) * 0.05)(B, S, D)), 'wqkv': _w((lambda *s: _rng.normal(s) * 0.05)(D, 3 * D)), 'wo': _w((lambda *s: _rng.normal(s) * 0.05)(D, D))}
    _A_in = _A_setup()

    def _B_setup():
        B, S, D, Dff = (1, 2048, 576, 4608)
        return {'x': _w((lambda *s: _rng.normal(s) * 0.05)(B, S, D)), 'w1': _w((lambda *s: _rng.normal(s) * 0.05)(D, Dff)), 'w2': _w((lambda *s: _rng.normal(s) * 0.05)(Dff, D))}
    _B_in = _B_setup()
    return {'A_x': _A_in['x'], 'A_wqkv': _A_in['wqkv'], 'A_wo': _A_in['wo'], 'B_x': _B_in['x'], 'B_w1': _B_in['w1'], 'B_w2': _B_in['w2'], 'c': _w((lambda *s: _rng.normal(s) * 0.05)(1, 576) * 8.0), 'w_mod': _w((lambda *s: _rng.normal(s) * 0.05)(576, 6 * 576) * 576 ** (-0.5) * 8.0)}

def reference(A_x, A_wqkv, A_wo, B_x, B_w1, B_w2, c, w_mod):

    def _A_ref(x, wqkv, wo):
        B, S, D = x.shape
        H = 32
        Dh = D // H
        W, dil = (8, 2)
        qkv = (lambda x, *d: x.transpose(*d))((x @ wqkv).reshape(B, S, 3, H, Dh), 2, 0, 3, 1, 4)
        q, k, v = (qkv[0], qkv[1], qkv[2])
        scale = Dh ** (-0.5)
        pos = jnp.arange(S)
        off = jnp.arange(W) * dil
        idx = pos[:, None] - off[None, :]
        mask = idx >= 0
        idx_c = jnp.where(mask, idx, 0).reshape(-1)
        kg = k[:, :, idx_c, :].reshape(B, H, S, W, Dh)
        vg = v[:, :, idx_c, :].reshape(B, H, S, W, Dh)
        logits = jnp.einsum('bhsd,bhswd->bhsw', q, kg) * scale
        logits = jnp.where(mask[None, None, :, :], logits, -1000000000.0)
        attn = _softmax(logits, axis=-1)
        o = jnp.einsum('bhsw,bhswd->bhsd', attn, vg)
        return (lambda x, *d: x.transpose(*d))(o, 0, 2, 1, 3).reshape(B, S, D) @ wo

    def _B_ref(x, w1, w2):
        h = jnp.einsum('bsd,df->bsf', x, w1)
        zero = jnp.zeros_like(h)
        h = jnp.maximum(h, zero)
        return jnp.einsum('bsf,fd->bsd', h, w2)
    x = A_x
    mod = (_silu(c) @ w_mod).reshape(c.shape[0], 6, 1, -1)
    sa, ca, ga, sb, cb, gb = (mod[:, 0].copy(), mod[:, 1].copy(), mod[:, 2].copy(), mod[:, 3].copy(), mod[:, 4].copy(), mod[:, 5].copy())
    h = _layernorm(x, axis=-1) * (1 + ca) + sa
    x = x + ga * _A_ref(h, A_wqkv, A_wo)
    h = _layernorm(x, axis=-1) * (1 + cb) + sb
    x = x + gb * _B_ref(h, B_w1, B_w2)
    return x
```

```python
import functools

import jax
import jax.numpy as jnp
import numpy as np
import jax.experimental.pallas as pl
import jax.experimental.pallas.tpu as pltpu

S = 2048
D = 576
DFF = 4608
H = 32
DH = 18
W = 8
DIL = 2
EPS = 1e-5
HALO = 16
NQ = 14
LOG2E = 1.4426950408889634
QSCALE = (DH ** -0.5) * LOG2E
NEG = -1e9 * LOG2E

TM = 256
TM2 = 256
TF = 512
F32 = jnp.float32
BF16 = jnp.bfloat16


def _qk_row0(t, d):
    if d < 16:
        tile, grp = {0: 0, 1: 5, 2: 9}[t] + d // 4, d % 4
    elif t == 0:
        tile, grp = 4, d - 16
    else:
        tile, grp = 13, (d - 16) + 2 * (t - 1)
    return tile * 128 + grp * 32


def _layernorm_mod(x, g, s):
    m = jnp.sum(x, axis=-1, keepdims=True) * (1.0 / D)
    xc = x - m
    v = jnp.sum(xc * xc, axis=-1, keepdims=True) * (1.0 / D)
    return (xc * jax.lax.rsqrt(v + EPS)) * g + s


def _kernel(x_hbm, wqkv_hbm, wo_hbm, w1_hbm, w2_hbm, c_hbm, wmod_hbm, out_hbm,
            x_v, wq_v, wqT_v, wp_v, wo_v, wof_v, wop_v, w1_v, w2_v, c_v, wmod_v, mod_v,
            q_p, q_q, kv_p, kv_q, x1_v, h2_v, out_v, sems, osem):
    cp_c = pltpu.make_async_copy(c_hbm, c_v, sems.at[0])
    cp_wmod = pltpu.make_async_copy(wmod_hbm, wmod_v, sems.at[1])
    cp_wq = pltpu.make_async_copy(wqkv_hbm, wq_v, sems.at[2])
    cp_x0 = pltpu.make_async_copy(x_hbm.at[pl.ds(0, TM)], x_v.at[pl.ds(0, TM)], sems.at[3])
    cp_x1 = pltpu.make_async_copy(x_hbm.at[pl.ds(TM, S - TM)], x_v.at[pl.ds(TM, S - TM)], sems.at[4])
    cp_wo = pltpu.make_async_copy(wo_hbm, wo_v, sems.at[5])
    cp_w1 = pltpu.make_async_copy(w1_hbm, w1_v, sems.at[6])
    cp_w2 = pltpu.make_async_copy(w2_hbm, w2_v, sems.at[7])
    cp_c.start()
    cp_wq.start()
    cp_wmod.start()
    cp_x0.start()
    cp_wo.start()
    cp_x1.start()
    cp_w1.start()
    cp_w2.start()

    for j in range(9):
        kv_p[j, pl.ds(0, HALO), :] = jnp.zeros((HALO, 128), F32)

    cp_wq.wait()
    for kb in range(5):
        kr = min(128, D - kb * 128)
        for nb in range(14):
            nr = min(128, 3 * D - nb * 128)
            blk = wq_v[pl.ds(kb * 128, kr), pl.ds(nb * 128, nr)].astype(F32)
            wqT_v[kb, pl.ds(nb * 128, nr), pl.ds(0, kr)] = blk.T
    for t in range(3):
        for d in range(DH):
            r0 = _qk_row0(t, d)
            for kb in range(5):
                kr = min(128, D - kb * 128)
                rows = wqT_v[kb, pl.ds(t * D + d, H, stride=DH), :]
                wp_v[pl.ds(r0, H), pl.ds(kb * 128, kr)] = rows[:, :kr].astype(BF16)
    wp_v[pl.ds(4 * 128 + 64, 64), :] = jnp.zeros((64, D), BF16)

    cp_wo.wait()
    for nb in range(5):
        nr = min(128, D - nb * 128)
        wof_v[nb, :, pl.ds(0, nr)] = wo_v[:, pl.ds(nb * 128, nr)].astype(F32)
    for d in range(DH):
        r0 = (d // 4) * 128 + (d % 4) * 32 if d < 16 else 4 * 128 + (d - 16 + 2) * 32
        for nb in range(5):
            nr = min(128, D - nb * 128)
            rows = wof_v[nb, pl.ds(d, H, stride=DH), :]
            wop_v[pl.ds(r0, H), pl.ds(nb * 128, nr)] = rows[:, :nr].astype(BF16)
    wop_v[pl.ds(4 * 128, 64), :] = jnp.zeros((64, D), BF16)

    cp_c.wait()
    cp_wmod.wait()
    cf = jnp.broadcast_to(c_v[...].astype(F32), (16, D))
    sc = (cf * jax.nn.sigmoid(cf)).astype(BF16)
    mod = jnp.dot(sc, wmod_v[...], preferred_element_type=F32)
    for j in range(6):
        mj = mod[:, j * D:(j + 1) * D]
        if j in (1, 4):
            mj = 1.0 + mj
        mod_v[j] = mj

    def stage_a(tile, q_ref, kv_ref, kv_prev):
        r0 = pl.multiple_of(tile * TM, TM)
        g = mod_v[1]
        s = mod_v[0]
        hs = []
        for gi in range(TM // 16):
            xg = x_v[pl.ds(r0 + gi * 16, 16), :].astype(F32)
            hs.append(_layernorm_mod(xg, g, s).astype(BF16))
        h = jnp.concatenate(hs, axis=0)
        res = jax.lax.dot_general(h, wp_v[...], (((1,), (1,)), ((), ())),
                                  preferred_element_type=F32)
        if kv_prev is not None:
            for j in range(9):
                kv_ref[j, pl.ds(0, HALO), :] = kv_prev[j, pl.ds(TM, HALO), :]
        for j in range(5):
            q_ref[j] = res[:, j * 128:(j + 1) * 128] * QSCALE
        for j in range(9):
            kv_ref[j, pl.ds(HALO, TM), :] = res[:, (5 + j) * 128:(6 + j) * 128]

    def attn_rows(tile, rt, q_ref, kv_ref):
        r = rt * 8
        qs = [q_ref[j, pl.ds(r, 8), :] for j in range(5)]
        ls = []
        for w in range(W):
            o = HALO + r - DIL * w
            a = qs[0] * kv_ref[0, pl.ds(o, 8), :]
            for j in range(1, 4):
                a = a + qs[j] * kv_ref[j, pl.ds(o, 8), :]
            a = a + qs[4] * kv_ref[8, pl.ds(o, 8), :]
            a = a + pltpu.roll(a, 64, 1)
            a = a + pltpu.roll(a, 32, 1)
            if r < DIL * w:
                pos = tile * TM + r + jax.lax.broadcasted_iota(jnp.int32, (8, 128), 0)
                a = jnp.where(pos >= DIL * w, a, NEG)
            ls.append(a)
        m = jnp.maximum(jnp.maximum(jnp.maximum(ls[0], ls[1]), jnp.maximum(ls[2], ls[3])),
                        jnp.maximum(jnp.maximum(ls[4], ls[5]), jnp.maximum(ls[6], ls[7])))
        ps = [jnp.exp2(l - m) for l in ls]
        den = ((ps[0] + ps[1]) + (ps[2] + ps[3])) + ((ps[4] + ps[5]) + (ps[6] + ps[7]))
        inv = 1.0 / den
        outs = []
        for j in range(5):
            acc = None
            for w in range(W):
                o = HALO + r - DIL * w
                term = ps[w] * kv_ref[4 + j, pl.ds(o, 8), :]
                acc = term if acc is None else acc + term
            outs.append(acc * inv)
        return outs

    def stage_b(tile, q_ref, kv_ref):
        og = []
        for gi in range(TM // 16):
            a = attn_rows(tile, 2 * gi, q_ref, kv_ref)
            b = attn_rows(tile, 2 * gi + 1, q_ref, kv_ref)
            og.append(jnp.concatenate(
                [jnp.concatenate([a[j], b[j]], axis=0).astype(BF16) for j in range(5)], axis=1))
        return jnp.concatenate(og, axis=0)

    def stage_c(tile, o):
        r0 = pl.multiple_of(tile * TM, TM)
        y = jnp.dot(o, wop_v[...], preferred_element_type=F32)
        ga = mod_v[2]
        g = mod_v[4]
        s = mod_v[3]
        for gi in range(TM // 16):
            rows = pl.ds(r0 + gi * 16, 16)
            x1 = x_v[rows, :].astype(F32) + ga * y[gi * 16:(gi + 1) * 16]
            x1_v[rows, :] = x1
            h2_v[rows, :] = _layernorm_mod(x1, g, s).astype(BF16)

    nt = S // TM
    cp_x0.wait()
    stage_a(0, q_p, kv_p, None)
    cp_x1.wait()

    def pair(p, carry):
        t0 = 2 * p
        o = stage_b(t0, q_p, kv_p)
        stage_a(t0 + 1, q_q, kv_q, kv_p)
        stage_c(t0, o)
        o = stage_b(t0 + 1, q_q, kv_q)
        stage_a(t0 + 2, q_p, kv_p, kv_q)
        stage_c(t0 + 1, o)
        return carry

    jax.lax.fori_loop(0, nt // 2 - 1, pair, 0)
    o = stage_b(nt - 2, q_p, kv_p)
    stage_a(nt - 1, q_q, kv_q, kv_p)
    stage_c(nt - 2, o)
    o = stage_b(nt - 1, q_q, kv_q)
    stage_c(nt - 1, o)

    cp_w1.wait()
    cp_w2.wait()
    nt2 = S // TM2

    def out_copy(i):
        rows = pl.ds(pl.multiple_of(i * TM2, TM2), TM2)
        return pltpu.make_async_copy(out_v.at[rows], out_hbm.at[rows], osem.at[i])

    def ffn(i, carry):
        r0 = pl.multiple_of(i * TM2, TM2)
        h2 = h2_v[pl.ds(r0, TM2), :]
        acc = None
        for j in range(DFF // TF):
            hid = jnp.dot(h2, w1_v[:, pl.ds(j * TF, TF)], preferred_element_type=F32)
            hid = jnp.maximum(hid, 0.0).astype(BF16)
            part = jnp.dot(hid, w2_v[pl.ds(j * TF, TF), :], preferred_element_type=F32)
            acc = part if acc is None else acc + part
        res = x1_v[pl.ds(r0, TM2), :] + mod_v[5][0:1] * acc
        out_v[pl.ds(r0, TM2), :] = res.astype(BF16)
        out_copy(i).start()
        return carry

    jax.lax.fori_loop(0, nt2, ffn, 0)
    for i in range(nt2):
        out_copy(i).wait()


@jax.jit
def pallas_adaLN_cond__sliding_local_dilated__dense_activation_relu__prompt_kernel(A_x, A_wqkv, A_wo, B_x, B_w1, B_w2, c, w_mod):
    x2 = A_x.reshape(S, D)
    any_spec = pl.BlockSpec(memory_space=pl.ANY)
    out = pl.pallas_call(
        _kernel,
        out_shape=jax.ShapeDtypeStruct((S, D), BF16),
        in_specs=[any_spec] * 7,
        out_specs=any_spec,
        scratch_shapes=[
            pltpu.VMEM((S, D), BF16),
            pltpu.VMEM((D, 3 * D), BF16),
            pltpu.VMEM((5, 3 * D, 128), F32),
            pltpu.VMEM((NQ * 128, D), BF16),
            pltpu.VMEM((D, D), BF16),
            pltpu.VMEM((5, D, 128), F32),
            pltpu.VMEM((640, D), BF16),
            pltpu.VMEM((D, DFF), BF16),
            pltpu.VMEM((DFF, D), BF16),
            pltpu.VMEM((1, D), BF16),
            pltpu.VMEM((D, 6 * D), BF16),
            pltpu.VMEM((6, 16, D), F32),
            pltpu.VMEM((5, TM, 128), F32),
            pltpu.VMEM((5, TM, 128), F32),
            pltpu.VMEM((9, HALO + TM, 128), F32),
            pltpu.VMEM((9, HALO + TM, 128), F32),
            pltpu.VMEM((S, D), F32),
            pltpu.VMEM((S, D), BF16),
            pltpu.VMEM((S, D), BF16),
            pltpu.SemaphoreType.DMA((8,)),
            pltpu.SemaphoreType.DMA((S // TM2,)),
        ],
        compiler_params=pltpu.CompilerParams(vmem_limit_bytes=100 * 1024 * 1024),
    )(x2, A_wqkv, A_wo, B_w1, B_w2, c, w_mod)
    return out.reshape(1, S, D)
```

```python
import jax
import jax.numpy as jnp
import jax.experimental.pallas as pl
import jax.experimental.pallas.tpu as pltpu

S = 2048
D = 576
DFF = 4608
H = 32
DH = 18
W = 8
DIL = 2
EPS = 1e-5

KP = 640
HALO = 16
NQ = 14
LOG2E = 1.4426950408889634
QSCALE = (DH ** -0.5) * LOG2E
NEG = -1e9 * LOG2E

TM = 256
CPT = TM // 128
NT = S // TM
NG = TM // 16
NCOL = S // 128
TF = 2304
G2M = 288

F32 = jnp.float32
BF16 = jnp.bfloat16
U32 = jnp.uint32


def _qkv_row0(t, d):
    if d < 16:
        tile, grp = {0: 0, 1: 5, 2: 9}[t] + d // 4, d % 4
    elif t == 0:
        tile, grp = 4, d - 16
    else:
        tile, grp = 13, (d - 16) + 2 * (t - 1)
    return tile * 128 + grp * 32


def _token(vals, zero):
    acc = None
    for v in vals:
        vi = pltpu.bitcast(v, jnp.int32)
        acc = vi if acc is None else acc | vi
    return acc & zero


def _after(x, tok):
    if tok is None:
        return x
    return pltpu.bitcast(pltpu.bitcast(x, jnp.int32) | tok, F32)


def _ln_stats(load, zero):
    nch = D // 16

    def colsum(vals):
        acc = [None] * 2
        for i, v in enumerate(vals):
            acc[i % 2] = v if acc[i % 2] is None else acc[i % 2] + v
        t = acc[0] + acc[1]
        t = t[0:8] + t[8:16]
        return jnp.sum(t, axis=0, keepdims=True)

    m = colsum([load(0, i) for i in range(nch)]) * (1.0 / D)
    sq = []
    for i in range(nch):
        xc = load(1, i) - m
        sq.append(xc * xc)
    v = colsum(sq) * (1.0 / D)
    rstd = jax.lax.rsqrt(v + EPS)
    m = _after(jnp.broadcast_to(m, (8, 128)), _token([jnp.broadcast_to(rstd, (8, 128))], zero))[0:1]
    return m, rstd


def _ln_mod(load, g, s, zero, stats=None):
    m, rstd = _ln_stats(load, zero) if stats is None else stats
    out = []
    for i in range(D // 16):
        out.append(((load(2, i) - m) * rstd) * g(i) + s(i))
    tok = _token([out[-1][8:16]], zero)
    out.append(jnp.zeros((KP - D, 128), F32))
    return jnp.concatenate(out, axis=0).astype(BF16).T, tok


def _pack(x):
    return pltpu.bitcast(x, U32)


def _load_mat(ref, rows=None, z=0):
    if ref.dtype == BF16:
        ref = ref.bitcast(U32)
    if rows is None:
        parts = [pltpu.bitcast(ref[kb + z], BF16) for kb in range(5)]
    else:
        parts = [pltpu.bitcast(ref[kb, rows, :], BF16) for kb in range(5)]
    return jnp.concatenate(parts, axis=1)


def _nt_dot(a, b):
    return jax.lax.dot_general(a, b, (((1,), (1,)), ((), ())), preferred_element_type=F32)


def _kernel(xt_hbm, wqkv_hbm, wo_hbm, w1_hbm, w2t_hbm, c_hbm, wmod_hbm, out_hbm,
            xt_v, wq_v, wqt_v, wp_v, wo_v, wof_v, wop_v, wopt_v, w1_v, w2t_v,
            c_v, wma_v, wmb_v, wmc_v, modt_v, modc_v, zero_v, o_v, h_a, h_b,
            q_p, q_q, kv_p, kv_q, x1t_v, h2_v, out_v, sems, xsem, osem):
    def col_copy(src, c0, cn, dst, sem):
        return pltpu.make_async_copy(src.at[:, pl.ds(c0, cn)], dst, sem)

    cp_c = pltpu.make_async_copy(c_hbm, c_v, sems.at[0])
    cp_wma = col_copy(wmod_hbm, 0, 2 * D, wma_v, sems.at[1])
    cp_wmb = col_copy(wmod_hbm, 9 * 128, 14 * 128, wmb_v, sems.at[2])
    cp_wmc = col_copy(wmod_hbm, 22 * 128, 5 * 128, wmc_v, sems.at[3])
    cp_wo = pltpu.make_async_copy(wo_hbm, wo_v, sems.at[4])
    cp_w1 = pltpu.make_async_copy(w1_hbm, w1_v, sems.at[5])
    cp_w2 = pltpu.make_async_copy(w2t_hbm, w2t_v, sems.at[6])
    wq_cols = [(0, 640), (640, 512), (1152, D)]
    cp_wq = [col_copy(wqkv_hbm, c0, cn, wq_v.at[:, pl.ds(c0, cn)], sems.at[7 + t])
             for t, (c0, cn) in enumerate(wq_cols)]
    cp_x = [col_copy(xt_hbm, j * 128, 128, xt_v.at[j], xsem.at[j]) for j in range(NCOL)]

    def out_copy(j):
        return pltpu.make_async_copy(
            out_v.at[j], out_hbm.at[:, pl.ds(pl.multiple_of(j * 128, 128), 128)], osem.at[j])

    cp_c.start(priority=0)
    for j in range(CPT):
        cp_x[j].start(priority=0)
    cp_wma.start(priority=1)

    zero_v[...] = jnp.zeros((8, 128), jnp.int32)
    for j in range(9):
        kv_p[j, pl.ds(0, HALO), :] = jnp.zeros((HALO, 128), F32)

    def mod_part(w_ref, dst, blk0, plus_one):
        cf = jnp.broadcast_to(c_v[...].astype(F32), (16, D))
        sc = (cf * jax.nn.sigmoid(cf)).astype(BF16)
        mod = jnp.dot(sc, w_ref[...], preferred_element_type=F32)[0:8]
        for nb in range(w_ref.shape[1] // 128):
            blk = mod[:, nb * 128:(nb + 1) * 128]
            dst[pl.ds((blk0 + nb) * 128, 128), :] = jnp.concatenate([blk] * 16, axis=0).T
        for j in plus_one:
            modt_v[pl.ds(j * D, D), :] = modt_v[pl.ds(j * D, D), :] + 1.0

    def prep_wq(t):
        c0, cn = wq_cols[t]
        for kb in range(5):
            kr = min(128, D - kb * 128)
            for nb in range(c0 // 128, (c0 + cn + 127) // 128):
                nr = min(128, 3 * D - nb * 128)
                blk = wq_v[pl.ds(kb * 128, kr), pl.ds(nb * 128, nr)].astype(F32)
                if kr < 128:
                    blk = jnp.concatenate([blk, jnp.zeros((128 - kr, nr), F32)], axis=0)
                wqt_v[kb, pl.ds(nb * 128, nr), :] = blk.T
        for kb in range(5):
            for d in range(DH):
                rows = wqt_v[kb, pl.ds(t * D + d, H, stride=DH), :]
                wp_v[kb, pl.ds(_qkv_row0(t, d), H), :] = rows.astype(BF16)
            if t == 0:
                wp_v[kb, pl.ds(4 * 128 + 64, 64), :] = jnp.zeros((64, 128), BF16)

    def prep_wo():
        for nb in range(5):
            nr = min(128, D - nb * 128)
            wof_v[nb, :, pl.ds(0, nr)] = wo_v[:, pl.ds(nb * 128, nr)].astype(F32)
        for d in range(DH):
            r0 = (d // 4) * 128 + (d % 4) * 32 if d < 16 else 4 * 128 + (d - 16 + 2) * 32
            for nb in range(5):
                nr = min(128, D - nb * 128)
                rows = wof_v[nb, pl.ds(d, H, stride=DH), :]
                wop_v[pl.ds(r0, H), pl.ds(nb * 128, nr)] = rows[:, :nr].astype(BF16)
        wop_v[pl.ds(4 * 128, 64), :] = jnp.zeros((64, D), BF16)
        wopt = wop_v[...].T
        for kb in range(5):
            wopt_v[kb] = _pack(wopt[:, kb * 128:(kb + 1) * 128])

    def mod_rows(j):
        return lambda i: modt_v[pl.ds(j * D + 16 * i, 16), :]

    def gate(x, tok):
        if tok is None:
            return x
        return jnp.concatenate([_after(x[0:8], tok), x[8:16]], axis=0)

    def x_loader(col, zs, tok):
        def load(p, i):
            x = xt_v.bitcast(U32)[col + zs[p], pl.ds(8 * i, 8), :]
            x = pltpu.bitcast(x, BF16).astype(F32)
            return gate(x, tok) if (p == 0 and i < 2) else x
        return load

    def ln1(col, zs, h_ref, cc, tok, stats=None):
        h, t = _ln_mod(x_loader(col, zs, tok), mod_rows(1), mod_rows(0), zero_v[...], stats)
        for kb in range(5):
            h_ref[kb, pl.ds(cc * 64, 64), :] = _pack(h[:, kb * 128:(kb + 1) * 128])
        return t

    def ln2(col, zs, tok):
        def load(p, i):
            x = x1t_v[col + zs[p], pl.ds(16 * i, 16), :]
            return gate(x, tok) if (p == 0 and i < 2) else x
        h, t = _ln_mod(load, mod_rows(4), mod_rows(3), zero_v[...])
        row0 = col * 64 if isinstance(col, int) else pl.multiple_of(col * 64, 64)
        for kb in range(5):
            h2_v[kb, pl.ds(row0, 64), :] = _pack(h[:, kb * 128:(kb + 1) * 128])
        return t

    def ln_jobs(t2, t1, h_ref, zs, gtoks, slots, order="2211"):
        queues = {"2": [("2", t2 * CPT + cc, cc) for cc in range(CPT)] if t2 is not None else [],
                  "1": [("1", t1 * CPT + cc, cc) for cc in range(CPT)] if t1 is not None else []}
        jobs = [queues[o].pop(0) for o in order if queues[o]]
        prev = None
        for k, (kind, col, cc) in enumerate(jobs):
            tok = prev
            if slots[k] >= 0:
                tok = gtoks[slots[k]] if tok is None else tok | gtoks[slots[k]]
            prev = ln2(col, zs, tok) if kind == "2" else ln1(col, zs, h_ref, cc, tok)

    def qkv(h_ref, q_ref, kv_ref, kv_prev, n0=0, n1=NQ):
        res = _nt_dot(_load_mat(h_ref), _load_mat(wp_v, pl.ds(n0 * 64, (n1 - n0) * 64)))
        if kv_prev is not None:
            for j in range(9):
                kv_ref[j, pl.ds(0, HALO), :] = kv_prev[j, pl.ds(TM, HALO), :]
        toks = []
        for n in range(n0, n1):
            r = res[:, (n - n0) * 128:(n - n0 + 1) * 128]
            if n < 5:
                q_ref[n] = r * QSCALE
            else:
                kv_ref[n - 5, pl.ds(HALO, TM), :] = r
            toks.append(_token([r[0:8]], zero_v[...]))
        return toks

    def attn_rows(tile, rt, q_ref, kv_ref, tok):
        r = rt * 8
        qs = [q_ref[j, pl.ds(r, 8), :] for j in range(5)]
        qs = [_after(q, tok) for q in qs]
        ls = []
        for w in range(W):
            o = HALO + r - DIL * w
            a = qs[0] * kv_ref[0, pl.ds(o, 8), :]
            for j in range(1, 4):
                a = a + qs[j] * kv_ref[j, pl.ds(o, 8), :]
            a = a + qs[4] * kv_ref[8, pl.ds(o, 8), :]
            a = a + pltpu.roll(a, 64, 1)
            a = a + pltpu.roll(a, 32, 1)
            if r < DIL * w:
                pos = tile * TM + r + jax.lax.broadcasted_iota(jnp.int32, (8, 128), 0)
                a = jnp.where(pos >= DIL * w, a, NEG)
            ls.append(a)
        m = jnp.maximum(jnp.maximum(jnp.maximum(ls[0], ls[1]), jnp.maximum(ls[2], ls[3])),
                        jnp.maximum(jnp.maximum(ls[4], ls[5]), jnp.maximum(ls[6], ls[7])))
        ps = [jnp.exp2(l - m) for l in ls]
        den = ((ps[0] + ps[1]) + (ps[2] + ps[3])) + ((ps[4] + ps[5]) + (ps[6] + ps[7]))
        inv = 1.0 / den
        outs = []
        for j in range(5):
            acc = None
            for w in range(W):
                o = HALO + r - DIL * w
                term = ps[w] * kv_ref[4 + j, pl.ds(o, 8), :]
                acc = term if acc is None else acc + term
            outs.append(acc * inv)
        return outs

    def attn_groups(tile, q_ref, kv_ref, o_ref, gates, toks, og, g0, g1):
        for gi in range(g0, g1):
            tok = gates(gi, toks)
            a = attn_rows(tile, 2 * gi, q_ref, kv_ref, tok)
            b = attn_rows(tile, 2 * gi + 1, q_ref, kv_ref, tok)
            packed = [jnp.concatenate([a[j], b[j]], axis=0).astype(BF16) for j in range(5)]
            if o_ref is not None:
                for j in range(5):
                    o_ref[j, pl.ds(16 * gi, 16), :] = packed[j]
            else:
                og.append(jnp.concatenate(packed, axis=1))
            toks.append(_token(packed, zero_v[...]))

    def paced(gtoks, nfree, g0, g1, span):
        def gates(gi, toks):
            if gi < nfree:
                return toks[gi - 1] if gi >= 1 else None
            tok = gtoks[min((gi - g0) * span // (g1 - g0), len(gtoks) - 1)]
            if gi >= 3:
                tok = tok | toks[gi - 3]
            return tok
        return gates

    def attn(tile, q_ref, kv_ref, gates, o_ref=None):
        og = []
        attn_groups(tile, q_ref, kv_ref, o_ref, gates, [], og, 0, NG)
        return None if o_ref is not None else jnp.concatenate(og, axis=0)

    def proj(tile, o):
        yt = jnp.concatenate(
            [_nt_dot(_load_mat(wopt_v, pl.ds(r // 2, G2M // 2)), o) for r in range(0, D, G2M)],
            axis=0)
        for cc in range(CPT):
            col = tile * CPT + cc
            xr = pltpu.bitcast(xt_v.bitcast(U32)[col], BF16)
            x1t_v[col] = xr.astype(F32) + modt_v[pl.ds(2 * D, D), :] * yt[:, cc * 128:(cc + 1) * 128]

    def ffn_chunk(h2, j, acc):
        hid = jnp.dot(h2, w1_v[:, pl.ds(j * TF, TF)], preferred_element_type=F32)
        hid = jnp.maximum(hid, 0.0).astype(BF16)
        part = _nt_dot(w2t_v[:, pl.ds(j * TF, TF)], hid)
        toks = [_token([hid[0:16, n * 128:(n + 1) * 128]], zero_v[...])
                for n in range(0, TF // 128, 2)]
        return (part if acc is None else acc + part), toks

    def ffn_out(i, acc):
        for cc in range(CPT):
            col = i * CPT + cc
            res = x1t_v[col] + modc_v[pl.ds(64, D), :] * acc[:, cc * 128:(cc + 1) * 128]
            out_v[col] = res.astype(BF16)
            out_copy(col).start()

    def load_h2(i):
        r0 = i * (TM // 2) if isinstance(i, int) else pl.multiple_of(i * (TM // 2), TM // 2)
        return _load_mat(h2_v, pl.ds(r0, TM // 2))[:, :D]

    zp = jax.lax.fori_loop(0, 2, lambda i, carry: carry + i, 0)
    z0 = (zp >> 10, zp >> 11, zp >> 12)
    cp_c.wait()
    cp_wq[0].start(priority=1)
    for j in range(CPT):
        cp_x[j].wait()
    cp_wq[1].start(priority=1)
    stats = [_ln_stats(x_loader(cc, z0, None), zero_v[...]) for cc in range(CPT)]
    cp_wma.wait()
    cp_wq[2].start(priority=1)
    for j in range(CPT, 2 * CPT):
        cp_x[j].start(priority=1)
    mod_part(wma_v, modt_v, 0, (1,))
    for cc in range(CPT):
        ln1(cc, z0, h_a, cc, None, stats[cc])
    cp_wq[0].wait()
    prep_wq(0)
    qkv(h_a, q_p, kv_p, None, 0, 2)
    cp_wq[1].wait()
    cp_wo.start(priority=1)
    cp_wmb.start(priority=1)
    qkv(h_a, q_p, kv_p, None, 2, 5)
    prep_wq(1)
    cp_wq[2].wait()
    for j in range(CPT, 2 * CPT):
        cp_x[j].wait()
    for j in range(2 * CPT, NCOL):
        cp_x[j].start(priority=1)
    qkv(h_a, q_p, kv_p, None, 5, 9)
    prep_wq(2)
    cp_wo.wait()
    cp_wmc.start(priority=1)
    cp_w1.start(priority=1)
    cp_w2.start(priority=1)
    g = qkv(h_a, q_p, kv_p, None, 9, NQ)
    ln_jobs(None, 1, h_b, z0, g, (-1, -1))
    prep_wo()
    og, toks = [], []
    g = qkv(h_b, q_q, kv_q, kv_p, 0, 7)
    attn_groups(0, q_p, kv_p, o_v, paced(g, 1, 1, 10, 6), toks, og, 0, 10)
    cp_wmb.wait()
    for j in range(2 * CPT, 3 * CPT):
        cp_x[j].wait()
    g = qkv(h_b, q_q, kv_q, None, 7, NQ)
    mod_part(wmb_v, modt_v, 9, (4,))
    attn_groups(0, q_p, kv_p, o_v, paced(g, 0, 10, NG, 5), toks, og, 10, NG)
    ln_jobs(None, 2, h_a, z0, g, (-1, 2))
    for j in range(3 * CPT, NCOL):
        cp_x[j].wait()

    def pair(p, carry):
        t = 2 * p + 1
        zs = (p >> 10, p >> 11, p >> 12)
        proj(t - 1, _load_mat(o_v, None, zs[0]))
        g = qkv(h_a, q_p, kv_p, kv_q)
        o = attn(t, q_q, kv_q, paced(g, 3, 3, NG, 12))
        ln_jobs(t - 1, t + 2, h_b, zs, g, (-1, 3, 7, 11), "1212")
        proj(t, o)
        g = qkv(h_b, q_q, kv_q, kv_p)
        attn(t + 1, q_p, kv_p, paced(g, 3, 3, NG, 12), o_v)
        ln_jobs(t, jnp.minimum(t + 3, NT - 1), h_a, zs, g, (-1, -1, 5, 9), "2211")
        return p

    pz = jax.lax.fori_loop(0, NT // 2 - 1, pair, 0)
    zt = (pz >> 10, pz >> 11, pz >> 12)
    cp_wmc.wait()
    cp_w1.wait()
    cp_w2.wait()

    proj(NT - 2, _load_mat(o_v, None, zt[0]))
    h2 = load_h2(0)
    acc, g = ffn_chunk(h2, 0, None)
    mod_part(wmc_v, modc_v, 0, ())
    o = attn(NT - 1, q_q, kv_q, paced(g, 6, 6, NG, 7))
    ln_jobs(NT - 2, None, None, zt, g, (-1, -1))
    proj(NT - 1, o)
    for j in range(1, DFF // TF):
        acc, g = ffn_chunk(h2, j, acc)
        if j == 1:
            ln_jobs(NT - 1, None, None, zt, g, (1, 4))
    ffn_out(0, acc)

    def ffn(i, carry):
        h2 = load_h2(i)
        acc = None
        for j in range(DFF // TF):
            acc, _ = ffn_chunk(h2, j, acc)
        ffn_out(i, acc)
        return carry

    jax.lax.fori_loop(1, NT, ffn, 0)
    for j in range(NCOL):
        out_copy(j).wait()


@jax.jit
def pallas_adaLN_cond__sliding_local_dilated__dense_activation_relu__prompt_kernel(A_x, A_wqkv, A_wo, B_x, B_w1, B_w2, c, w_mod):
    del B_x
    xt = A_x.reshape(S, D).T
    w2t = B_w2.T
    hbm = pl.BlockSpec(memory_space=pltpu.HBM)
    out_t = pl.pallas_call(
        _kernel,
        out_shape=jax.ShapeDtypeStruct((D, S), BF16),
        in_specs=[hbm] * 7,
        out_specs=hbm,
        scratch_shapes=[
            pltpu.VMEM((NCOL, D, 128), BF16),
            pltpu.VMEM((D, 3 * D), BF16),
            pltpu.VMEM((5, 3 * D, 128), F32),
            pltpu.VMEM((5, NQ * 128, 128), BF16),
            pltpu.VMEM((D, D), BF16),
            pltpu.VMEM((5, D, 128), F32),
            pltpu.VMEM((KP, D), BF16),
            pltpu.VMEM((5, D // 2, 128), U32),
            pltpu.VMEM((D, DFF), BF16),
            pltpu.VMEM((D, DFF), BF16),
            pltpu.VMEM((1, D), BF16),
            pltpu.VMEM((D, 2 * D), BF16),
            pltpu.VMEM((D, 14 * 128), BF16),
            pltpu.VMEM((D, 5 * 128), BF16),
            pltpu.VMEM((23 * 128, 128), F32),
            pltpu.VMEM((5 * 128, 128), F32),
            pltpu.VMEM((8, 128), jnp.int32),
            pltpu.VMEM((5, TM, 128), BF16),
            pltpu.VMEM((5, TM // 2, 128), U32),
            pltpu.VMEM((5, TM // 2, 128), U32),
            pltpu.VMEM((5, TM, 128), F32),
            pltpu.VMEM((5, TM, 128), F32),
            pltpu.VMEM((9, HALO + TM, 128), F32),
            pltpu.VMEM((9, HALO + TM, 128), F32),
            pltpu.VMEM((NCOL, D, 128), F32),
            pltpu.VMEM((5, S // 2, 128), U32),
            pltpu.VMEM((NCOL, D, 128), BF16),
            pltpu.SemaphoreType.DMA((10,)),
            pltpu.SemaphoreType.DMA((NCOL,)),
            pltpu.SemaphoreType.DMA((NCOL,)),
        ],
        compiler_params=pltpu.CompilerParams(
            vmem_limit_bytes=100 * 1024 * 1024, disable_semaphore_checks=True),
    )(xt, A_wqkv, A_wo, B_w1, w2t, c, w_mod)
    return out_t.T.reshape(1, S, D)
```
